```python
import os as _os
_os.environ.setdefault("JAX_PLATFORMS", "cpu")
import jax
import jax.numpy as jnp

def _softmax(x, axis=-1):
    return jax.nn.softmax(x, axis=axis)
def _gelu(x):
    return jax.nn.gelu(x, approximate=True)
def _silu(x):
    return jax.nn.silu(x)
def _sigmoid(x):
    return jax.nn.sigmoid(x)
def _layernorm(x, axis=-1, eps=1e-5):
    m = jnp.mean(x, axis=axis, keepdims=True)
    v = jnp.var(x, axis=axis, keepdims=True)
    return (x - m) / jnp.sqrt(v + eps)
def _scatter_add(tgt, idx, src, axis=0):
    return tgt.at[idx].add(src)
def _segment_sum(src, seg, n):
    return jax.ops.segment_sum(src, seg, n)
class _Rng:
    def __init__(self, key):
        self._k = key
    def _next(self):
        self._k, sub = jax.random.split(self._k)
        return sub
    def normal(self, shape):
        return jax.random.normal(self._next(), shape, dtype=jnp.bfloat16)
    def randint(self, lo, hi, shape):
        return jax.random.randint(self._next(), shape, lo, hi, dtype=jnp.int32)
    def uniform(self, shape, lo=0.0, hi=1.0):
        return jax.random.uniform(self._next(), shape, jnp.bfloat16, lo, hi)
    def permutation(self, n):
        return jax.random.permutation(self._next(), n)


kernel_name = 'concat_heads__gqa_block_cached__gqa_block_cached__near_ridge'

def setup_inputs():
    _rng = _Rng(jax.random.key(int.from_bytes(__import__("os").urandom(4), "little")))
    _w = (lambda a: (lambda t: t.astype(jnp.bfloat16) if jnp.issubdtype(t.dtype, jnp.floating) else t)(jnp.asarray(a)))
    def _A_setup():
        B, Sq, D = 16, 144, 448
        Hq, Hkv, Sk, Dh = 16, 8, 1024, 256
        assert Hq % Hkv == 0, (Hq, Hkv)
        return {
            "x": _w((lambda *s: _rng.normal(s) * 0.8)(B, Sq, D)),
            "k_cache": _w((lambda *s: _rng.normal(s) * 0.8)(B, Hkv, Sk, Dh)),
            "v_cache": _w((lambda *s: _rng.normal(s) * 0.05)(B, Hkv, Sk, Dh)),
            "wq": _w((lambda *s: _rng.normal(s) * 0.8)(D, Hq * Dh) * (D ** -0.5)),
            "wo": _w((lambda *s: _rng.normal(s) * 0.05)(Hq * Dh, D) * ((Hq * Dh) ** -0.5)),
        }
    _A_in = _A_setup()

    def _B_setup():
        B, Sq, D = 16, 144, 448
        Hq, Hkv, Sk, Dh = 16, 8, 1024, 256
        assert Hq % Hkv == 0, (Hq, Hkv)
        return {
            "x": _w((lambda *s: _rng.normal(s) * 0.8)(B, Sq, D)),
            "k_cache": _w((lambda *s: _rng.normal(s) * 0.8)(B, Hkv, Sk, Dh)),
            "v_cache": _w((lambda *s: _rng.normal(s) * 0.05)(B, Hkv, Sk, Dh)),
            "wq": _w((lambda *s: _rng.normal(s) * 0.8)(D, Hq * Dh) * (D ** -0.5)),
            "wo": _w((lambda *s: _rng.normal(s) * 0.05)(Hq * Dh, D) * ((Hq * Dh) ** -0.5)),
        }
    _B_in = _B_setup()

    return {
        "A_x": _A_in["x"],
        "A_k_cache": _A_in["k_cache"],
        "A_v_cache": _A_in["v_cache"],
        "A_wq": _A_in["wq"],
        "A_wo": _A_in["wo"],
        "B_x": _B_in["x"],
        "B_k_cache": _B_in["k_cache"],
        "B_v_cache": _B_in["v_cache"],
        "B_wq": _B_in["wq"],
        "B_wo": _B_in["wo"],
    }

def reference(A_x, A_k_cache, A_v_cache, A_wq, A_wo, B_x, B_k_cache, B_v_cache, B_wq, B_wo):
    def _A_ref(x, k_cache, v_cache, wq, wo):
        B, Sq, D = x.shape
        Hq, Dh = 16, 256
        Hkv = k_cache.shape[1]
        rep = Hq // Hkv
        q = (lambda x, *d: x.transpose(*d))((x @ wq).reshape(B, Sq, Hq, Dh), 0, 2, 1, 3)
        k = jnp.repeat(k_cache, rep, axis=1)
        v = jnp.repeat(v_cache, rep, axis=1)
        scores = jnp.einsum("bhqd,bhkd->bhqk", q, k) * (Dh ** -0.5)
        p = _softmax(scores, axis=-1)
        o = jnp.einsum("bhqk,bhkd->bhqd", p, v)
        return (lambda x, *d: x.transpose(*d))(o, 0, 2, 1, 3).reshape(B, Sq, Hq * Dh) @ wo

    def _B_ref(x, k_cache, v_cache, wq, wo):
        B, Sq, D = x.shape
        Hq, Dh = 16, 256
        Hkv = k_cache.shape[1]
        rep = Hq // Hkv
        q = (lambda x, *d: x.transpose(*d))((x @ wq).reshape(B, Sq, Hq, Dh), 0, 2, 1, 3)
        k = jnp.repeat(k_cache, rep, axis=1)
        v = jnp.repeat(v_cache, rep, axis=1)
        scores = jnp.einsum("bhqd,bhkd->bhqk", q, k) * (Dh ** -0.5)
        p = _softmax(scores, axis=-1)
        o = jnp.einsum("bhqk,bhkd->bhqd", p, v)
        return (lambda x, *d: x.transpose(*d))(o, 0, 2, 1, 3).reshape(B, Sq, Hq * Dh) @ wo

    a = _A_ref(A_x, A_k_cache, A_v_cache, A_wq, A_wo)
    b = _B_ref(B_x, B_k_cache, B_v_cache, B_wq, B_wo)
    return jnp.concatenate([a, b], axis=-1)
```

```python
import jax
import jax.numpy as jnp
from jax import lax
import jax.experimental.pallas as pl
import jax.experimental.pallas.tpu as pltpu

B, SQ, D = 16, 144, 448
HQ, HKV, SK, DH = 16, 8, 1024, 256
G = 8
T = G * SQ
NJ = T // 128
NGRP = (B // G) * 2
C = 1.4426950408889634 / 16.0
NT = (((1,), (1,)), ((), ()))
QH = 2
PRE = True
RCP = 1
FLAGS = None
LP = {"XLA_TPU_FORCE_LP_LLO_SCHEDULER": True}
EV = {"XLA_TPU_EVENLY_DISTRIBUTE_CRITICAL_NODES": True}
SUMBF = False
FLAGS = LP
BC = 1
START_AT = 0
WO = 1
NP = {'XLA_TPU_MAX_INSTS_TO_PREDICATE': 4}


def mk(order, klag=1, olag=2):
    def prog(G, NJ):
        ops = [('k', u) for u in range(klag)]
        done = 0
        for u in range(G):
            for c in order:
                if c == 'k' and u + klag < G:
                    ops.append(('k', u + klag))
                elif c == 'v':
                    ops.append(('v', u))
                elif c == 'o' and u - olag >= 0:
                    ops.append(('o', u - olag)); done = u - olag + 1
        ops += [('o', j) for j in range(done, NJ)]
        return ops
    return prog


def txt(t):
    return lambda G, NJ: [(w[0], int(w[1:])) for w in t.split()]


PROG = mk('kov')


def _half(rows):
    if isinstance(rows, slice):
        return rows
    return pl.ds(rows.start // 2, rows.size // 2)


def _ld(ref, idx, rows=slice(None)):
    if BC == 0:
        return ref[(*idx, rows, slice(None))]
    r = ref.bitcast(jnp.uint32) if BC == 1 else ref
    return pltpu.bitcast(r[(*idx, _half(rows), slice(None))], jnp.bfloat16)


def _st(ref, idx, rows, val):
    if BC <= 1:
        ref[(*idx, rows, slice(None))] = val
    else:
        r = ref.bitcast(jnp.uint32) if BC == 1 else ref
        r[(*idx, _half(rows), slice(None))] = pltpu.bitcast(val, jnp.uint32)


def _dst(ref):
    return ref.bitcast(jnp.bfloat16) if BC == 2 else ref


def _buf(*shape):
    if BC == 2:
        return pltpu.VMEM((*shape[:-2], shape[-2] // 2, shape[-1]), jnp.uint32)
    return pltpu.VMEM(shape, jnp.bfloat16)


def _lanes(ref, idx, rows, n, first=0):
    return jnp.concatenate([_ld(ref, (*idx, first + c), rows) for c in range(n)], axis=1)


def _kernel(xa, ka, va, wqa, woa, xb, kb, vb, wqb, wob, out,
            kbuf, vbuf, xbuf, wqbuf, wobuf, q_scr, o_scr, acc, stage,
            kvsem, xsem, wqsem, osem, w_scr):
    def kvo_copies(k_hbm, v_hbm, wo_hbm, i):
        g, h, slot = i >> 4, i & 7, i & 1
        bs = pl.ds(g * G, G)
        cps = []
        for c in range(2):
            cps.append(pltpu.make_async_copy(k_hbm.at[bs, h, :, pl.ds(c * 128, 128)], _dst(kbuf).at[slot, c], kvsem.at[slot, c]))
        for c in range(2):
            cps.append(pltpu.make_async_copy(v_hbm.at[bs, h, :, pl.ds(c * 128, 128)], _dst(vbuf).at[slot, c], kvsem.at[slot, 2 + c]))
        if WO == 0:
            for c in range(4):
                cols = pl.ds(pl.multiple_of(h * 2 * DH + c * 128, 128), 128)
                cps.append(pltpu.make_async_copy(wo_hbm.at[:, cols], _dst(wobuf).at[slot, c], kvsem.at[slot, 4 + c]))
        else:
            cols = pl.ds(pl.multiple_of(h * 2 * DH, 2 * DH), 2 * DH)
            cps.append(pltpu.make_async_copy(wo_hbm.at[:, cols], wobuf.at[slot], kvsem.at[slot, 4]))
        return cps

    def wq_copy(wq_hbm, h):
        cols = pl.ds(h * 2 * DH if isinstance(h, int) else pl.multiple_of(h * 2 * DH, 2 * DH), 2 * DH)
        return pltpu.make_async_copy(wq_hbm.at[:, cols], wqbuf.at[h], wqsem.at[h])

    def x_copy(x_hbm, g):
        return pltpu.make_async_copy(x_hbm.at[pl.ds(g * T, T)], xbuf, xsem.at[0])

    def out_copy(g, j):
        return pltpu.make_async_copy(stage.at[pl.ds(j * 128, 128)], out.at[pl.ds(g * T + j * 128, 128)], osem.at[j])

    x_copy(xa, 0).start()
    for h in range(QH):
        wq_copy(wqa, h).start()
    x_copy(xa, 0).wait()
    for h in range(QH):
        wq_copy(wqa, h).wait()
    for h in range(QH, HKV):
        wq_copy(wqa, h).start()

    def group(grp, carry):
        g, br = grp >> 1, grp & 1

        @pl.when(grp > 0)
        def _():
            x_copy(xa, g).wait()

        def qphase(t, carry):
            @pl.when(grp + t > 0)
            def _():
                for r in range(QH):
                    wq_copy(wqa, t * QH + r).wait()

            @pl.when(jnp.logical_and(grp == 0, t == 1))
            def _():
                for c in kvo_copies(ka, va, woa, grp):
                    c.start()

            for r in range(QH):
                h = t * QH + r
                qf = jnp.dot(xbuf[...], wqbuf[h], preferred_element_type=jnp.float32)
                qb = ((qf * C) if PRE else qf).astype(jnp.bfloat16)
                for c in range(4):
                    _st(q_scr, (h, c), slice(None), qb[:, c * 128:(c + 1) * 128])
            return carry

        lax.fori_loop(0, HKV // QH, qphase, 0)

        def body(h, carry):
            i = grp * HKV + h
            slot = h & 1
            nxt = i + 1
            nbr = (nxt >> 3) & 1
            more = grp + 1 < NGRP

            def starts():
                @pl.when(jnp.logical_and(nxt < NGRP * HKV, nbr == 0))
                def _():
                    for c in kvo_copies(ka, va, woa, nxt):
                        c.start()

                @pl.when(nbr == 1)
                def _():
                    for c in kvo_copies(kb, vb, wob, nxt):
                        c.start()

                @pl.when(br == 0)
                def _():
                    wq_copy(wqb, h).start()

                    @pl.when(h == 0)
                    def _():
                        x_copy(xb, g).start()

                @pl.when(jnp.logical_and(br == 1, more))
                def _():
                    wq_copy(wqa, h).start()

                    @pl.when(h == 0)
                    def _():
                        x_copy(xa, g + 1).start()

            for c in kvo_copies(ka, va, woa, i):
                c.wait()
            if START_AT == 0:
                starts()

            def qk(u):
                rows = pl.ds(u * SQ, SQ)
                q2 = jnp.concatenate([_lanes(q_scr, (h,), rows, 2, 0), _lanes(q_scr, (h,), rows, 2, 2)], axis=0)
                k = jnp.concatenate([_ld(kbuf, (slot, 0, u)), _ld(kbuf, (slot, 1, u))], axis=1)
                return lax.dot_general(q2, k, NT, preferred_element_type=jnp.float32)

            def softmax(s):
                m = jnp.max(s, axis=-1, keepdims=True)
                p = jnp.exp2(s - m) if PRE else jnp.exp2((s - m) * C)
                pb = p.astype(jnp.bfloat16)
                l = jnp.sum(pb.astype(jnp.float32) if SUMBF else p, axis=-1, keepdims=True)
                if RCP == 0:
                    r = 1.0 / l
                else:
                    r = pl.reciprocal(l, approx=True)
                    for _ in range(RCP):
                        r = r * (2.0 - l * r)
                return pb, r

            def pv(u, p, r):
                v = jnp.concatenate([_ld(vbuf, (slot, 0, u)), _ld(vbuf, (slot, 1, u))], axis=1)
                o = (jnp.dot(p, v, preferred_element_type=jnp.float32) * r).astype(jnp.bfloat16)
                rows = pl.ds(u * SQ, SQ)
                for e in range(2):
                    for c in range(2):
                        _st(o_scr, (2 * e + c,), rows, o[e * SQ:(e + 1) * SQ, c * 128:(c + 1) * 128])

            def oproj(j):
                cols = pl.ds(j * 128, 128)
                rows = pl.ds(pl.multiple_of(br * D, D), D)
                if WO == 0:
                    w = _lanes(wobuf, (slot,), slice(None), 4)
                elif WO == 1:
                    w = wobuf[slot]
                else:
                    w = _lanes(w_scr, (), slice(None), 4)
                o = _lanes(o_scr, (), cols, 4)
                y = lax.dot_general(w, o, NT, preferred_element_type=jnp.float32)
                acc[rows, cols] = jnp.where(h == 0, 0.0, acc[rows, cols]) + y

            if WO == 2:
                for c in range(4):
                    w_scr[c] = wobuf[slot, :, c * 128:(c + 1) * 128]
            S = {}
            for n, (op, u) in enumerate(PROG(G, NJ)):
                if n == START_AT and n > 0:
                    starts()
                if op == 'k':
                    S[u] = qk(u)
                elif op == 'v':
                    pv(u, *softmax(S.pop(u)))
                elif op == 'o':
                    oproj(u)
            return carry

        lax.fori_loop(0, HKV, body, 0)

        @pl.when(br == 1)
        def _():
            @pl.when(g > 0)
            def _():
                for j in range(NJ):
                    out_copy(g - 1, j).wait()
            for j in range(NJ):
                stage[pl.ds(j * 128, 128), :] = acc[:, pl.ds(j * 128, 128)].T.astype(jnp.bfloat16)
                out_copy(g, j).start()
        return carry

    lax.fori_loop(0, NGRP, group, 0)
    for j in range(NJ):
        out_copy(B // G - 1, j).wait()


@jax.jit
def pallas_concat_heads__gqa_block_cached__gqa_block_cached__near_ridge_kernel(A_x, A_k_cache, A_v_cache, A_wq, A_wo, B_x, B_k_cache, B_v_cache, B_wq, B_wo):
    hbm = pl.BlockSpec(memory_space=pltpu.HBM)
    bf = jnp.bfloat16
    out = pl.pallas_call(
        _kernel,
        in_specs=[hbm] * 10,
        out_specs=hbm,
        out_shape=jax.ShapeDtypeStruct((B * SQ, 2 * D), bf),
        scratch_shapes=[
            _buf(2, 2, G, SK, 128), _buf(2, 2, G, SK, 128),
            pltpu.VMEM((T, D), bf),
            pltpu.VMEM((HKV, D, 2 * DH), bf), _buf(2, 4, D, 128) if WO == 0 else pltpu.VMEM((2, D, 2 * DH), bf),
            _buf(HKV, 4, T, 128), _buf(4, T, 128),
            pltpu.VMEM((2 * D, T), jnp.float32), pltpu.VMEM((T, 2 * D), bf),
            pltpu.SemaphoreType.DMA((2, 8)), pltpu.SemaphoreType.DMA((1,)),
            pltpu.SemaphoreType.DMA((HKV,)),
            pltpu.SemaphoreType.DMA((NJ,)), pltpu.VMEM((4, D, 128), bf),
        ],
        compiler_params=pltpu.CompilerParams(vmem_limit_bytes=100 * 1024 * 1024,
                                             disable_bounds_checks=True, flags=FLAGS),
    )(A_x.reshape(B * SQ, D), A_k_cache, A_v_cache, A_wq, A_wo.T,
      B_x.reshape(B * SQ, D), B_k_cache, B_v_cache, B_wq, B_wo.T)
    return out.reshape(B, SQ, 2 * D)
```

```python
import jax
import jax.numpy as jnp
from jax import lax
import jax.experimental.pallas as pl
import jax.experimental.pallas.tpu as pltpu

B, SQ, D = 16, 144, 448
HKV, SK, DH = 8, 1024, 256
G = 8
T = G * SQ
NJ = T // 128
NG = B // G
HB = 2
NS = HKV // HB
NB = 2 * NS
SH = NS.bit_length() - 1
HW = 2 * DH
W = HB * HW
NC = 2 * D // 128
NCA = D // 128
QSCALE = 1.4426950408889634 * DH ** -0.5
NT = (((1,), (1,)), ((), ()))
Q_ROWS = (128, 80, 80)
O_ROWS = (224, 224)


def _program():
    n_units, n_o = G * HB, NJ * HB * len(O_ROWS)

    def last_unit_of(piece):
        r, j = divmod(piece // len(O_ROWS), NJ)
        return r * G + min(j, G - 1)

    ops, done = [("k", 0)], 0
    for w in range(n_units):
        for op in "aobocv":
            if op in "abc":
                if w + 1 < n_units:
                    ops.append((op, w + 1))
            elif op == "v":
                ops.append((op, w))
            elif last_unit_of(done) < w:
                ops.append(("o", done))
                done += 1
    return ops + [("o", piece) for piece in range(done, n_o)]


def _ld(ref, idx, start=0, size=None):
    size = ref.shape[-2] if size is None else size
    words = ref.bitcast(jnp.uint32)[(*idx, pl.ds(start // 2, size // 2), slice(None))]
    return pltpu.bitcast(words, jnp.bfloat16)


def _cat(parts, axis):
    return jnp.concatenate(parts, axis=axis)


def _kernel(xa, ka, va, wqa, woa, xb, kb, vb, wqb, wob, out,
            kbuf, vbuf, xbuf, wqbuf, wobuf, q_scr, o_scr, acc, stage,
            kvsem, xsem, wqsem, wosem, osem, psem):

    def kv_copies(k_hbm, v_hbm, g, t, slot):
        bs, hs = pl.ds(g * G, G), pl.ds(t * HB, HB)
        return [pltpu.make_async_copy(src.at[bs, hs, :, pl.ds(c * 128, 128)], dst.at[slot, c],
                                      kvsem.at[slot, 2 * n + c])
                for n, (src, dst) in enumerate(((k_hbm, kbuf), (v_hbm, vbuf))) for c in range(2)]

    def wq_copy(wq_hbm, t, n):
        return pltpu.make_async_copy(wq_hbm.at[:, pl.ds(t * W, W)], wqbuf.at[n], wqsem.at[n])

    def wo_copies():
        return [pltpu.make_async_copy(wo_hbm.at[:, pl.ds(t * W + c * 128, 128)],
                                      wobuf.at[br * NS + t, c], wosem.at[0])
                for br, wo_hbm in enumerate((woa, wob)) for t in range(NS) for c in range(W // 128)]

    def x_copy(x_hbm, g, br):
        return pltpu.make_async_copy(x_hbm.at[pl.ds(g * T, T)], xbuf.at[br], xsem.at[br])

    def out_copy(g, c):
        return pltpu.make_async_copy(stage.at[c], out.at[pl.ds(g * T, T), pl.ds(c * 128, 128)],
                                     osem.at[c])

    def transpose_out(c):
        rows = pl.ds(c * 128 if isinstance(c, int) else pl.multiple_of(c * 128, 128), 128)
        for j in range(NJ):
            tok = pl.ds(j * 128, 128)
            stage[c, tok, :] = acc[rows, tok].T.astype(jnp.bfloat16)

    def qproj(n, r, tok=pl.ds(0, T)):
        qf = jnp.dot(xbuf[n >> SH, tok, :], wqbuf[n, :, r * HW:(r + 1) * HW],
                     preferred_element_type=jnp.float32)
        qb = (qf * QSCALE).astype(jnp.bfloat16)
        for c in range(HW // 128):
            q_scr[n, 4 * r + c, tok, :] = qb[:, c * 128:(c + 1) * 128]

    ts = T // 2
    x0 = [pltpu.make_async_copy(xa.at[pl.ds(i * ts, ts)], xbuf.at[0, pl.ds(i * ts, ts)], psem.at[i])
          for i in range(2)]
    w0 = [pltpu.make_async_copy(wqa.at[:, pl.ds(r * HW, HW)], wqbuf.at[0, :, pl.ds(r * HW, HW)],
                                psem.at[2 + r]) for r in range(HB)]
    x0[0].start()
    w0[0].start()
    acc[...] = jnp.zeros(acc.shape, acc.dtype)
    x0[0].wait()
    w0[0].wait()
    for c in x0[1:] + w0[1:]:
        c.start()
    qproj(0, 0, pl.ds(0, ts))
    x0[1].wait()
    for t in range(1, NS):
        wq_copy(wqa, t, t).start()
    qproj(0, 0, pl.ds(ts, ts))
    x_copy(xb, 0, 1).start()
    for t in range(NS):
        wq_copy(wqb, t, NS + t).start()
    for r in range(1, HB):
        w0[r].wait()
        qproj(0, r)
    for c in kv_copies(ka, va, 0, 0, 0) + wo_copies():
        c.start()

    def group(grp, carry):
        g, br = grp >> 1, grp & 1

        def q_step(n, carry):
            @pl.when(grp == 0)
            def _():
                wq_copy(wqa, 0, n).wait()

                @pl.when(n == NS)
                def _():
                    x_copy(xa, 0, 1).wait()

            for r in range(HB):
                transpose_out(jnp.minimum(HB * (n & (NS - 1)) + r, NC - 1))
                qproj(n, r)
            return carry

        @pl.when(g > 0)
        def _():
            x_copy(xa, g, br).wait()

            @pl.when(br == 1)
            def _():
                for c in range(NC):
                    out_copy(g, c).wait()

        lo = jnp.where(grp == 0, 1, jnp.where(grp == 1, NB, br * NS))
        hi = jnp.where(grp == 0, NB, (br + 1) * NS)
        lax.fori_loop(lo, hi, q_step, 0)

        @pl.when(grp == 0)
        def _():
            for c in kv_copies(ka, va, 0, 0, 0) + wo_copies():
                c.wait()
            for c in kv_copies(ka, va, 0, 1, 1):
                c.start()
            x_copy(xa, 1, 0).start()
            x_copy(xb, 1, 1).start()

        @pl.when(grp == 2)
        def _():
            for c in range(NC):
                out_copy(0, c).start()

        @pl.when(grp == 3)
        def _():
            for c in range(NCA):
                out_copy(1, c).start()

        def body(t, carry):
            slot = t & 1
            n = br * NS + t

            def scores(w, piece):
                r, u = divmod(w, G)
                q = _cat([_cat([_ld(q_scr, (n, 4 * r + 2 * h + c), u * SQ, SQ) for c in range(2)], 1)
                          for h in range(2)], 0)
                if piece is not None:
                    q = q[sum(Q_ROWS[:piece]):sum(Q_ROWS[:piece + 1])]
                k = _cat([_ld(kbuf, (slot, c, u, r)) for c in range(2)], 1)
                return lax.dot_general(q, k, NT, preferred_element_type=jnp.float32)

            def softmax(s):
                m = s[:, :128]
                for c in range(128, SK, 128):
                    m = jnp.maximum(m, s[:, c:c + 128])
                m = jnp.max(m, axis=-1, keepdims=True)
                p = jnp.exp2(s - m)
                l = jnp.sum(p, axis=-1, keepdims=True)
                inv = pl.reciprocal(l, approx=True)
                inv = inv * (2.0 - l * inv)
                return p.astype(jnp.bfloat16), inv

            def attend(w, p, inv):
                r, u = divmod(w, G)
                v = _cat([_ld(vbuf, (slot, c, u, r)) for c in range(2)], 1)
                o = (jnp.dot(p, v, preferred_element_type=jnp.float32) * inv).astype(jnp.bfloat16)
                for h in range(2):
                    for c in range(2):
                        o_scr[4 * r + 2 * h + c, pl.ds(u * SQ, SQ), :] = (
                            o[h * SQ:(h + 1) * SQ, c * 128:(c + 1) * 128])

            def oproj(piece):
                tile, part = divmod(piece, len(O_ROWS))
                r, j = divmod(tile, NJ)
                cols = pl.ds(j * 128, 128)
                d0, dn = sum(O_ROWS[:part]), O_ROWS[part]
                rows = pl.ds(pl.multiple_of(br * D + d0, 16), dn)
                o = _cat([_ld(o_scr, (4 * r + c,), j * 128, 128) for c in range(4)], 1)
                wt = _cat([_ld(wobuf, (n, 4 * r + c), d0, dn) for c in range(4)], 1)
                y = lax.dot_general(wt, o, NT, preferred_element_type=jnp.float32)
                if r == 0:
                    acc[rows, cols] = jnp.where(t == 0, 0.0, acc[rows, cols]) + y
                else:
                    acc[rows, cols] = acc[rows, cols] + y

            s = {}
            for op, w in _program():
                if op == "k":
                    s[w] = scores(w, None)
                elif op == "a":
                    s[w] = scores(w, 0)
                elif op in "bc":
                    s[w] = _cat([s[w], scores(w, "abc".index(op))], 0)
                elif op == "v":
                    attend(w, *softmax(s.pop(w)))
                else:
                    oproj(w)

            i2 = grp * NS + t + 2
            g2, br2, t2 = i2 >> (SH + 1), (i2 >> SH) & 1, i2 & (NS - 1)

            @pl.when(jnp.logical_and(g2 < NG, br2 == 0))
            def _():
                for c in kv_copies(ka, va, g2, t2, slot):
                    c.start()

            @pl.when(br2 == 1)
            def _():
                for c in kv_copies(kb, vb, g2, t2, slot):
                    c.start()

            @pl.when(i2 - 1 < NG * NB)
            def _():
                for c in kv_copies(ka, va, 0, 0, 1 - slot):
                    c.wait()
            return carry

        lax.fori_loop(0, NS, body, 0)
        return carry

    lax.fori_loop(0, 2 * NG, group, 0)
    for c in range(NCA, NC):
        transpose_out(c)
        out_copy(NG - 1, c).start()
    for c in range(NC):
        out_copy(NG - 1, c).wait()


@jax.jit
def pallas_concat_heads__gqa_block_cached__gqa_block_cached__near_ridge_kernel(
    A_x: jax.Array,
    A_k_cache: jax.Array,
    A_v_cache: jax.Array,
    A_wq: jax.Array,
    A_wo: jax.Array,
    B_x: jax.Array,
    B_k_cache: jax.Array,
    B_v_cache: jax.Array,
    B_wq: jax.Array,
    B_wo: jax.Array,
):
    hbm = pl.BlockSpec(memory_space=pltpu.HBM)
    bf = jnp.bfloat16
    out = pl.pallas_call(
        _kernel,
        in_specs=[hbm] * 10,
        out_specs=hbm,
        out_shape=jax.ShapeDtypeStruct((B * SQ, 2 * D), bf),
        scratch_shapes=[
            pltpu.VMEM((2, 2, G, HB, SK, 128), bf),
            pltpu.VMEM((2, 2, G, HB, SK, 128), bf),
            pltpu.VMEM((2, T, D), bf),
            pltpu.VMEM((NB, D, W), bf),
            pltpu.VMEM((NB, W // 128, D, 128), bf),
            pltpu.VMEM((NB, W // 128, T, 128), bf),
            pltpu.VMEM((W // 128, T, 128), bf),
            pltpu.VMEM((2 * D, T), jnp.float32),
            pltpu.VMEM((NC, T, 128), bf),
            pltpu.SemaphoreType.DMA((2, 4)),
            pltpu.SemaphoreType.DMA((2,)),
            pltpu.SemaphoreType.DMA((NB,)),
            pltpu.SemaphoreType.DMA((1,)),
            pltpu.SemaphoreType.DMA((NC,)),
            pltpu.SemaphoreType.DMA((2 + HB,)),
        ],
        compiler_params=pltpu.CompilerParams(
            vmem_limit_bytes=110 * 1024 * 1024,
            flags={"XLA_TPU_FORCE_LP_LLO_SCHEDULER": True},
        ),
    )(A_x.reshape(B * SQ, D), A_k_cache, A_v_cache, A_wq, A_wo.T,
      B_x.reshape(B * SQ, D), B_k_cache, B_v_cache, B_wq, B_wo.T)
    return out.reshape(B, SQ, 2 * D)
```

```python
import jax
import jax.numpy as jnp
from jax import lax
import jax.experimental.pallas as pl
import jax.experimental.pallas.tpu as pltpu

B, SQ, D = 16, 144, 448
HKV, SK, DH = 8, 1024, 256
G = 8
T = G * SQ
NJ = T // 128
NG = B // G
HB = 2
NS = HKV // HB
NB = 2 * NS
SH = NS.bit_length() - 1
HW = 2 * DH
W = HB * HW
NC = 2 * D // 128
NCA = D // 128
QSCALE = 1.4426950408889634 * DH ** -0.5
NT = (((1,), (1,)), ((), ()))
QH = 3
Q_ROWS = (128, 80, 80)
O_ROWS = (224, 224)


def _program():
    n_units, n_o = G * HB, NJ * HB * len(O_ROWS)

    def last_unit_of(piece):
        r, j = divmod(piece // len(O_ROWS), NJ)
        return r * G + min(j, G - 1)

    ops, done = [("k", 0)], 0
    for w in range(n_units):
        for op in "aobocv":
            if op in "abc":
                if w + 1 < n_units:
                    ops.append((op, w + 1))
            elif op == "v":
                ops.append((op, w))
            elif last_unit_of(done) < w:
                ops.append(("o", done))
                done += 1
    return ops + [("o", piece) for piece in range(done, n_o)]


def _ld(ref, idx, start=0, size=None):
    size = ref.shape[-2] if size is None else size
    words = ref.bitcast(jnp.uint32)[(*idx, pl.ds(start // 2, size // 2), slice(None))]
    return pltpu.bitcast(words, jnp.bfloat16)


def _cat(parts, axis):
    return jnp.concatenate(parts, axis=axis)


def _kernel(xa, ka, va, wqa, woa, xb, kb, vb, wqb, wob, out,
            kbuf, vbuf, xbuf, wqbuf, wobuf, q_scr, o_scr, acc, stage,
            kvsem, xsem, wqsem, wosem, osem, psem):

    def kv_copies(k_hbm, v_hbm, g, t, slot):
        bs, hs = pl.ds(g * G, G), pl.ds(t * HB, HB)
        return [pltpu.make_async_copy(src.at[bs, hs, :, pl.ds(c * 128, 128)], dst.at[slot, c],
                                      kvsem.at[slot, 2 * n + c])
                for n, (src, dst) in enumerate(((k_hbm, kbuf), (v_hbm, vbuf))) for c in range(2)]

    def wq_copy(wq_hbm, h, n):
        return pltpu.make_async_copy(wq_hbm.at[:, pl.ds(h * HW, HW)], wqbuf.at[n], wqsem.at[n])

    def wo_copies():
        return [pltpu.make_async_copy(wo_hbm.at[:, pl.ds(t * W + c * 128, 128)],
                                      wobuf.at[br * NS + t, c], wosem.at[0])
                for br, wo_hbm in enumerate((woa, wob)) for t in range(NS) for c in range(W // 128)]

    def x_copy(x_hbm, g, grp):
        return pltpu.make_async_copy(x_hbm.at[pl.ds(g * T, T)], xbuf.at[grp], xsem.at[grp])

    def out_copy(g, c):
        return pltpu.make_async_copy(stage.at[c], out.at[pl.ds(g * T, T), pl.ds(c * 128, 128)],
                                     osem.at[c])

    def transpose_out(c):
        rows = pl.ds(c * 128 if isinstance(c, int) else pl.multiple_of(c * 128, 128), 128)
        for j in range(NJ):
            tok = pl.ds(j * 128, 128)
            stage[c, tok, :] = acc[rows, tok].T.astype(jnp.bfloat16)

    def qproj(hh, tok=pl.ds(0, T)):
        qf = jnp.dot(xbuf[hh >> 3, tok, :], wqbuf[hh & (2 * HKV - 1)], preferred_element_type=jnp.float32)
        qb = (qf * QSCALE).astype(jnp.bfloat16)
        for c in range(HW // 128):
            q_scr[hh, c, tok, :] = qb[:, c * 128:(c + 1) * 128]

    ts = T // 2
    x0 = [pltpu.make_async_copy(xa.at[pl.ds(i * ts, ts)], xbuf.at[0, pl.ds(i * ts, ts)], psem.at[i])
          for i in range(2)]
    x0[0].start()
    wq_copy(wqa, 0, 0).start()

    @pl.loop(0, 2 * D // 64)
    def _(i):
        acc[pl.ds(pl.multiple_of(i * 64, 64), 64), :] = jnp.zeros((64, T), acc.dtype)

    x0[0].wait()
    wq_copy(wqa, 0, 0).wait()
    x0[1].start()
    wq_copy(wqa, 1, 1).start()

    @pl.loop(0, 4)
    def _(i):
        @pl.when(i == 1)
        def _():
            x0[1].wait()
            for h in range(2, HKV):
                wq_copy(wqa, h, h).start()

        @pl.when(i == 2)
        def _():
            wq_copy(wqa, 1, 1).wait()

        qproj(i >> 1, pl.ds(pl.multiple_of((i & 1) * ts, ts), ts))

    x_copy(xb, 0, 1).start()
    for h in range(HKV):
        wq_copy(wqb, h, HKV + h).start()
    x_copy(xa, 1, 2).start()
    for c in kv_copies(ka, va, 0, 0, 0) + wo_copies():
        c.start()

    def group(grp, carry):
        g, br = grp >> 1, grp & 1
        lo = jnp.where(grp == 0, 0, jnp.where(grp == 3, 8, 5))
        hi = jnp.where(grp <= 1, 5, jnp.where(grp == 2, 8, 10))

        def q_step(i, carry):
            for e in range(QH):
                hh = 2 + QH * i + e

                @pl.when(hh < 2 * HKV)
                def _():
                    wq_copy(wqa, 0, hh).wait()

                @pl.when((hh & (HKV - 1)) == 0)
                def _():
                    x_copy(xa, 0, hh >> 3).wait()

            for e in range(QH):
                transpose_out(jnp.minimum(QH * (i - lo) + e, NC - 1))
                qproj(2 + QH * i + e)
            return carry

        @pl.when(grp == 3)
        def _():
            for c in range(NC):
                out_copy(0, c).wait()

        lax.fori_loop(lo, hi, q_step, 0)

        @pl.when(grp == 0)
        def _():
            for c in kv_copies(ka, va, 0, 0, 0) + wo_copies():
                c.wait()
            for c in kv_copies(ka, va, 0, 1, 1):
                c.start()
            x_copy(xb, 1, 3).start()

        @pl.when(grp == 2)
        def _():
            for c in range(NC):
                out_copy(0, c).start()

        @pl.when(grp == 3)
        def _():
            for c in range(NCA):
                out_copy(1, c).start()

        def body(t, carry):
            slot = t & 1
            n = br * NS + t

            def scores(w, piece):
                r, u = divmod(w, G)
                q = _cat([_cat([_ld(q_scr, (grp * HKV + t * HB + r, 2 * h + c), u * SQ, SQ) for c in range(2)], 1)
                          for h in range(2)], 0)
                if piece is not None:
                    q = q[sum(Q_ROWS[:piece]):sum(Q_ROWS[:piece + 1])]
                k = _cat([_ld(kbuf, (slot, c, u, r)) for c in range(2)], 1)
                return lax.dot_general(q, k, NT, preferred_element_type=jnp.float32)

            def softmax(s):
                m = s[:, :128]
                for c in range(128, SK, 128):
                    m = jnp.maximum(m, s[:, c:c + 128])
                m = jnp.max(m, axis=-1, keepdims=True)
                p = jnp.exp2(s - m)
                l = jnp.sum(p, axis=-1, keepdims=True)
                inv = pl.reciprocal(l, approx=True)
                inv = inv * (2.0 - l * inv)
                return p.astype(jnp.bfloat16), inv

            def attend(w, p, inv):
                r, u = divmod(w, G)
                v = _cat([_ld(vbuf, (slot, c, u, r)) for c in range(2)], 1)
                o = (jnp.dot(p, v, preferred_element_type=jnp.float32) * inv).astype(jnp.bfloat16)
                for h in range(2):
                    for c in range(2):
                        o_scr[4 * r + 2 * h + c, pl.ds(u * SQ, SQ), :] = (
                            o[h * SQ:(h + 1) * SQ, c * 128:(c + 1) * 128])

            def oproj(piece):
                tile, part = divmod(piece, len(O_ROWS))
                r, j = divmod(tile, NJ)
                cols = pl.ds(j * 128, 128)
                d0, dn = sum(O_ROWS[:part]), O_ROWS[part]
                rows = pl.ds(pl.multiple_of(br * D + d0, 16), dn)
                o = _cat([_ld(o_scr, (4 * r + c,), j * 128, 128) for c in range(4)], 1)
                wt = _cat([_ld(wobuf, (n, 4 * r + c), d0, dn) for c in range(4)], 1)
                y = lax.dot_general(wt, o, NT, preferred_element_type=jnp.float32)
                if r == 0:
                    acc[rows, cols] = jnp.where(t == 0, 0.0, acc[rows, cols]) + y
                else:
                    acc[rows, cols] = acc[rows, cols] + y

            s = {}
            for op, w in _program():
                if op == "k":
                    s[w] = scores(w, None)
                elif op == "a":
                    s[w] = scores(w, 0)
                elif op in "bc":
                    s[w] = _cat([s[w], scores(w, "abc".index(op))], 0)
                elif op == "v":
                    attend(w, *softmax(s.pop(w)))
                else:
                    oproj(w)

            i2 = grp * NS + t + 2
            g2, br2, t2 = i2 >> (SH + 1), (i2 >> SH) & 1, i2 & (NS - 1)

            @pl.when(jnp.logical_and(g2 < NG, br2 == 0))
            def _():
                for c in kv_copies(ka, va, g2, t2, slot):
                    c.start()

            @pl.when(br2 == 1)
            def _():
                for c in kv_copies(kb, vb, g2, t2, slot):
                    c.start()

            @pl.when(i2 - 1 < NG * NB)
            def _():
                for c in kv_copies(ka, va, 0, 0, 1 - slot):
                    c.wait()
            return carry

        lax.fori_loop(0, NS, body, 0)
        return carry

    lax.fori_loop(0, 2 * NG, group, 0)
    for c in range(NCA, NC):
        transpose_out(c)
        out_copy(NG - 1, c).start()
    for c in range(NC):
        out_copy(NG - 1, c).wait()


@jax.jit
def pallas_concat_heads__gqa_block_cached__gqa_block_cached__near_ridge_kernel(
    A_x: jax.Array,
    A_k_cache: jax.Array,
    A_v_cache: jax.Array,
    A_wq: jax.Array,
    A_wo: jax.Array,
    B_x: jax.Array,
    B_k_cache: jax.Array,
    B_v_cache: jax.Array,
    B_wq: jax.Array,
    B_wo: jax.Array,
):
    hbm = pl.BlockSpec(memory_space=pltpu.HBM)
    bf = jnp.bfloat16
    out = pl.pallas_call(
        _kernel,
        in_specs=[hbm] * 10,
        out_specs=hbm,
        out_shape=jax.ShapeDtypeStruct((B * SQ, 2 * D), bf),
        scratch_shapes=[
            pltpu.VMEM((2, 2, G, HB, SK, 128), bf),
            pltpu.VMEM((2, 2, G, HB, SK, 128), bf),
            pltpu.VMEM((2 * NG, T, D), bf),
            pltpu.VMEM((2 * HKV, D, HW), bf),
            pltpu.VMEM((NB, W // 128, D, 128), bf),
            pltpu.VMEM((2 * NG * HKV, HW // 128, T, 128), bf),
            pltpu.VMEM((W // 128, T, 128), bf),
            pltpu.VMEM((2 * D, T), jnp.float32),
            pltpu.VMEM((NC, T, 128), bf),
            pltpu.SemaphoreType.DMA((2, 4)),
            pltpu.SemaphoreType.DMA((2 * NG,)),
            pltpu.SemaphoreType.DMA((2 * HKV,)),
            pltpu.SemaphoreType.DMA((1,)),
            pltpu.SemaphoreType.DMA((NC,)),
            pltpu.SemaphoreType.DMA((2,)),
        ],
        compiler_params=pltpu.CompilerParams(
            vmem_limit_bytes=120 * 1024 * 1024,
            flags={"XLA_TPU_FORCE_LP_LLO_SCHEDULER": True},
        ),
    )(A_x.reshape(B * SQ, D), A_k_cache, A_v_cache, A_wq, A_wo.T,
      B_x.reshape(B * SQ, D), B_k_cache, B_v_cache, B_wq, B_wo.T)
    return out.reshape(B, SQ, 2 * D)
```
